```python
import os as _os
_os.environ.setdefault("JAX_PLATFORMS", "cpu")
import jax
import jax.numpy as jnp

def _softmax(x, axis=-1):
    return jax.nn.softmax(x, axis=axis)
def _gelu(x):
    return jax.nn.gelu(x, approximate=True)
def _silu(x):
    return jax.nn.silu(x)
def _sigmoid(x):
    return jax.nn.sigmoid(x)
def _layernorm(x, axis=-1, eps=1e-5):
    m = jnp.mean(x, axis=axis, keepdims=True)
    v = jnp.var(x, axis=axis, keepdims=True)
    return (x - m) / jnp.sqrt(v + eps)
def _scatter_add(tgt, idx, src, axis=0):
    return tgt.at[idx].add(src)
def _segment_sum(src, seg, n):
    return jax.ops.segment_sum(src, seg, n)
class _Rng:
    def __init__(self, key):
        self._k = key
    def _next(self):
        self._k, sub = jax.random.split(self._k)
        return sub
    def normal(self, shape):
        return jax.random.normal(self._next(), shape, dtype=jnp.bfloat16)
    def randint(self, lo, hi, shape):
        return jax.random.randint(self._next(), shape, lo, hi, dtype=jnp.int32)
    def uniform(self, shape, lo=0.0, hi=1.0):
        return jax.random.uniform(self._next(), shape, jnp.bfloat16, lo, hi)
    def permutation(self, n):
        return jax.random.permutation(self._next(), n)


kernel_name = 'gated_mix__linear_kernel_hedgehog__glu_gated_bilinear__prompt'

def setup_inputs():
    _rng = _Rng(jax.random.key(int.from_bytes(__import__("os").urandom(4), "little")))
    _w = (lambda a: (lambda t: t.astype(jnp.bfloat16) if jnp.issubdtype(t.dtype, jnp.floating) else t)(jnp.asarray(a)))
    def _A_setup():
        B, S, D, H = 1, 2048, 512, 32
        Dh = D // H
        return {
            "x": _w((lambda *s: _rng.normal(s) * 0.05)(B, S, D)),
            "wqkv": _w((lambda *s: _rng.normal(s) * 0.8)(D, 3 * D)),
            "w_phi": _w((lambda *s: _rng.normal(s) * 0.8)(H, Dh, Dh) * (Dh ** -0.5)),
            "wo": _w((lambda *s: _rng.normal(s) * 0.05)(D, D)),
        }
    _A_in = _A_setup()

    def _B_setup():
        B, S, D, F = 1, 2048, 512, 1792
        return {
            "x": _w((lambda *s: _rng.normal(s) * 0.05)(B, S, D)),
            "w_gate": _w((lambda *s: _rng.normal(s) * 1.6)(D, F) * (D ** -0.5)),
            "w_up": _w((lambda *s: _rng.normal(s) * 1.6)(D, F) * (D ** -0.5)),
            "w_down": _w((lambda *s: _rng.normal(s) * 1.6)(F, D) * (F ** -0.5)),
        }
    _B_in = _B_setup()

    return {
        "A_x": _A_in["x"],
        "A_wqkv": _A_in["wqkv"],
        "A_w_phi": _A_in["w_phi"],
        "A_wo": _A_in["wo"],
        "B_x": _B_in["x"],
        "B_w_gate": _B_in["w_gate"],
        "B_w_up": _B_in["w_up"],
        "B_w_down": _B_in["w_down"],
        "gate_w": _w((lambda *s: _rng.normal(s) * 0.05)(512) * 16.0),
    }

def reference(A_x, A_wqkv, A_w_phi, A_wo, B_x, B_w_gate, B_w_up, B_w_down, gate_w):
    def _A_ref(x, wqkv, w_phi, wo):
        B, S, D = x.shape
        H = 32; Dh = D // H
        qkv = (lambda x, *d: x.transpose(*d))((x @ wqkv).reshape(B, S, 3, H, Dh), 2, 0, 3, 1, 4)
        q, k, v = qkv[0], qkv[1], qkv[2]
        pq = jnp.einsum("bhsd,hdf->bhsf", q, w_phi)
        pk = jnp.einsum("bhsd,hdf->bhsf", k, w_phi)
        phi_q = jnp.concatenate([_softmax(pq, axis=-1), _softmax(-pq, axis=-1)], axis=-1)
        phi_k = jnp.concatenate([_softmax(pk, axis=-1), _softmax(-pk, axis=-1)], axis=-1)
        kv = jnp.einsum("bhsf,bhsd->bhfd", phi_k, v)
        z  = jnp.einsum("bhsf->bhf", phi_k)
        num = jnp.einsum("bhqf,bhfd->bhqd", phi_q, kv)
        den = jnp.einsum("bhqf,bhf->bhq", phi_q, z)[..., None] + 1e-6
        o = num / den
        return (lambda x, *d: x.transpose(*d))(o, 0, 2, 1, 3).reshape(B, S, D) @ wo

    def _B_ref(x, w_gate, w_up, w_down):
        g = jnp.einsum("bsd,df->bsf", x, w_gate)
        u = jnp.einsum("bsd,df->bsf", x, w_up)
        h = g * u
        return jnp.einsum("bsf,fd->bsd", h, w_down)

    x = A_x
    g = _sigmoid((x * gate_w).sum(-1, keepdims=True))
    a = _A_ref(x, A_wqkv, A_w_phi, A_wo)
    b = _B_ref(x, B_w_gate, B_w_up, B_w_down)
    return g * a + (1 - g) * b
```

```python
import jax
import jax.numpy as jnp
import jax.experimental.pallas as pl
import jax.experimental.pallas.tpu as pltpu

_H = 32
_DH = 16
_G = 4
_LOG2E = 1.4426950408889634
_T = 512
_U = 1024
_OC = 4

_NT = (((1,), (1,)), ((), ()))
_TN = (((0,), (0,)), ((), ()))


def _iota(shape, dim):
    return jax.lax.broadcasted_iota(jnp.int32, shape, dim)


def _dual_softmax(pt):
    s = [pt[8 * f:8 * (f + 1)] for f in range(_DH)]
    mx, mn = s[0], s[0]
    for f in range(1, _DH):
        mx = jnp.maximum(mx, s[f])
        mn = jnp.minimum(mn, s[f])
    out = []
    for e in ([jnp.exp2(a - mx) for a in s], [jnp.exp2(mn - a) for a in s]):
        tot = e[0]
        for f in range(1, _DH):
            tot = tot + e[f]
        r = 1.0 / tot
        out += [a * r for a in e]
    return out


def _kernel(x_hbm, wqkv_hbm, wphi_hbm, gw_hbm, wo_hbm, wg_hbm, wu_hbm, wd_hbm,
            o_hbm,
            x_ref, wqkv_ref, wphi_ref, gw_ref, wt_ref, lhs_ref, kv_ref, z_ref,
            wo_ref, wg_ref, wu_ref, wd_ref, o_ref, sems, osems):
    f32, bf16 = jnp.float32, jnp.bfloat16
    S, D = x_ref.shape
    T = _T
    nt = S // T
    U = _U
    nu = S // U
    C = U // _OC

    def rows(i, n):
        return pl.ds(i * n, n)

    cx = [pltpu.make_async_copy(x_hbm.at[rows(i, T)], x_ref.at[rows(i, T)], sems.at[i])
          for i in range(nt)]
    cw = [pltpu.make_async_copy(wqkv_hbm.at[:, rows(w, D)], wqkv_ref.at[w], sems.at[nt + w])
          for w in range(3)]
    rest = [pltpu.make_async_copy(src, dst, sems.at[nt + 3 + n]) for n, (src, dst) in enumerate(
        [(wphi_hbm, wphi_ref), (gw_hbm, gw_ref), (wo_hbm, wo_ref),
         (wg_hbm, wg_ref), (wu_hbm, wu_ref), (wd_hbm, wd_ref)])]
    rest[0].start()
    cw[1].start()
    cx[0].start()
    cw[2].start()

    rest[0].wait()
    e = (_iota((_H, D), 0) == _iota((_H, D), 1) // _DH).astype(bf16)
    a = jnp.dot(wphi_ref[...], e, preferred_element_type=f32)
    a = jnp.where(_iota((256, D), 0) // _DH == _iota((256, D), 1) % _DH, a, 0.0).astype(bf16)
    r = (_iota((128, 256), 0) // 8 == _iota((128, 256), 1) % _DH).astype(bf16)
    mt = jnp.dot(r, a, preferred_element_type=f32)
    mt = jnp.where(_iota((128, D), 0) % 8 == (_iota((128, D), 1) // _DH) % 8, mt, 0.0).astype(bf16)

    def fold(w):
        for g in range(_G):
            sl = slice(128 * g, 128 * (g + 1))
            t = jax.lax.dot_general(mt[:, sl], wqkv_ref[w, :, sl], _NT, preferred_element_type=f32)
            wt_ref[w, sl, :] = (t * _LOG2E).astype(bf16)

    def proj(w, g, x):
        return jax.lax.dot_general(wt_ref[w, 128 * g:128 * (g + 1), :], x, _NT,
                                   preferred_element_type=f32)

    kv_ref[...] = jnp.zeros(kv_ref.shape, f32)
    z_ref[...] = jnp.zeros(z_ref.shape, f32)
    cw[1].wait()
    fold(1)
    cw[2].wait()
    for c in cx[1:] + [cw[0]] + rest[1:]:
        c.start()

    def kv_body(i, carry):
        base = pl.ds(pl.multiple_of(i * T, T), T)
        pltpu.make_async_copy(x_hbm.at[base], x_ref.at[base], sems.at[i]).wait()
        x = x_ref[base, :]
        pk = [proj(1, g, x) for g in range(_G)]
        v = jnp.dot(x, wqkv_ref[2], preferred_element_type=f32).astype(bf16)
        for g in range(_G):
            phik = _dual_softmax(pk[g])
            z_ref[g] += jnp.concatenate(
                [sum(a[:, 128 * c:128 * (c + 1)] for c in range(1, T // 128)) + a[:, :128]
                 for a in phik], axis=0)
            phik = jnp.concatenate(phik, axis=0).astype(bf16)
            kv_ref[g] += jnp.dot(phik, v[:, 128 * g:128 * (g + 1)], preferred_element_type=f32)
        return carry

    jax.lax.fori_loop(0, nt, kv_body, 0)
    cw[0].wait()
    fold(0)
    own = _iota((128, 256), 0) // _DH == _iota((128, 256), 1) % 8
    ownz = _iota((16, 256), 0) == _iota((16, 256), 1) % 8
    for g in range(_G):
        kvt = jnp.where(own, kv_ref[g].T, 0.0)
        zrow = jnp.sum(z_ref[g], axis=1, keepdims=True)
        zt = jnp.where(ownz, jnp.broadcast_to(zrow, (256, 128)).T[:16], 0.0)
        lhs_ref[g] = jnp.concatenate([kvt, zt], axis=0).astype(bf16)
    for c in rest[1:]:
        c.wait()

    def out_copy(n):
        return pltpu.make_async_copy(o_ref.at[rows(n, C)], o_hbm.at[rows(n, C)], osems.at[n])

    def body(i, carry):
        base = pl.multiple_of(i * U, U)
        x = x_ref[pl.ds(base, U), :]
        gate = jax.nn.sigmoid(jnp.sum(
            x.astype(f32) * gw_ref[...].reshape(1, D).astype(f32), axis=1, keepdims=True))
        ots = []
        for g in range(_G):
            phiq = jnp.concatenate(_dual_softmax(proj(0, g, x)), axis=0).astype(bf16)
            r = jnp.dot(lhs_ref[g], phiq, preferred_element_type=f32)
            inv = 1.0 / (r[128:136] + 1e-6)
            ots += [r[8 * k:8 * (k + 1)] * inv[k // 2:k // 2 + 1] for k in range(16)]
        ot = jnp.concatenate(ots, axis=0).astype(bf16)
        a = jax.lax.dot_general(ot, wo_ref[...], _TN, preferred_element_type=f32)
        hg = jnp.dot(x, wg_ref[...], preferred_element_type=f32)
        hu = jnp.dot(x, wu_ref[...], preferred_element_type=f32)
        h = (hg * hu).astype(bf16)
        for c in range(_OC):
            sl = slice(c * C, (c + 1) * C)
            b = jnp.dot(h[sl], wd_ref[...], preferred_element_type=f32)
            o_ref[pl.ds(base + c * C, C), :] = (
                gate[sl] * a[sl] + (1.0 - gate[sl]) * b).astype(o_ref.dtype)
            out_copy(i * _OC + c).start()
        return carry

    jax.lax.fori_loop(0, nu, body, 0)
    for n in range(nu * _OC):
        out_copy(n).wait()


@jax.jit
def pallas_gated_mix__linear_kernel_hedgehog__glu_gated_bilinear__prompt_kernel(
    A_x: jax.Array,
    A_wqkv: jax.Array,
    A_w_phi: jax.Array,
    A_wo: jax.Array,
    B_x: jax.Array,
    B_w_gate: jax.Array,
    B_w_up: jax.Array,
    B_w_down: jax.Array,
    gate_w: jax.Array,
):
    del B_x
    B, S, D = A_x.shape
    F = B_w_gate.shape[1]
    nt = S // _T
    bf16 = jnp.bfloat16
    hbm = pl.BlockSpec(memory_space=pl.ANY)
    out = pl.pallas_call(
        _kernel,
        in_specs=[hbm] * 8,
        out_specs=hbm,
        out_shape=jax.ShapeDtypeStruct((S, D), A_x.dtype),
        scratch_shapes=[
            pltpu.VMEM((S, D), bf16),
            pltpu.VMEM((3, D, D), bf16),
            pltpu.VMEM((_DH * _DH, _H), bf16),
            pltpu.VMEM((D,), bf16),
            pltpu.VMEM((2, D, D), bf16),
            pltpu.VMEM((_G, 144, 256), bf16),
            pltpu.VMEM((_G, 256, 128), jnp.float32),
            pltpu.VMEM((_G, 256, 128), jnp.float32),
            pltpu.VMEM((D, D), bf16),
            pltpu.VMEM((D, F), bf16),
            pltpu.VMEM((D, F), bf16),
            pltpu.VMEM((F, D), bf16),
            pltpu.VMEM((S, D), A_x.dtype),
            pltpu.SemaphoreType.DMA((nt + 9,)),
            pltpu.SemaphoreType.DMA((S // _U * _OC,)),
        ],
        compiler_params=pltpu.CompilerParams(vmem_limit_bytes=100 * 1024 * 1024),
    )(A_x.reshape(S, D), A_wqkv, A_w_phi.transpose(1, 2, 0).reshape(_DH * _DH, _H), gate_w,
      A_wo, B_w_gate, B_w_up, B_w_down)
    return out.reshape(B, S, D)
```
